```python
import os as _os
_os.environ.setdefault("JAX_PLATFORMS", "cpu")
import jax
import jax.numpy as jnp

def _softmax(x, axis=-1):
    return jax.nn.softmax(x, axis=axis)
def _gelu(x):
    return jax.nn.gelu(x, approximate=True)
def _silu(x):
    return jax.nn.silu(x)
def _sigmoid(x):
    return jax.nn.sigmoid(x)
def _layernorm(x, axis=-1, eps=1e-5):
    m = jnp.mean(x, axis=axis, keepdims=True)
    v = jnp.var(x, axis=axis, keepdims=True)
    return (x - m) / jnp.sqrt(v + eps)
def _scatter_add(tgt, idx, src, axis=0):
    return tgt.at[idx].add(src)
def _segment_sum(src, seg, n):
    return jax.ops.segment_sum(src, seg, n)
class _Rng:
    def __init__(self, key):
        self._k = key
    def _next(self):
        self._k, sub = jax.random.split(self._k)
        return sub
    def normal(self, shape):
        return jax.random.normal(self._next(), shape, dtype=jnp.bfloat16)
    def randint(self, lo, hi, shape):
        return jax.random.randint(self._next(), shape, lo, hi, dtype=jnp.int32)
    def uniform(self, shape, lo=0.0, hi=1.0):
        return jax.random.uniform(self._next(), shape, jnp.bfloat16, lo, hi)
    def permutation(self, n):
        return jax.random.permutation(self._next(), n)


kernel_name = 'standalone__gqa_softmax__decode'

def setup_inputs():
    _rng = _Rng(jax.random.key(int.from_bytes(__import__("os").urandom(4), "little")))
    _w = (lambda a: (lambda t: t.astype(jnp.bfloat16) if jnp.issubdtype(t.dtype, jnp.floating) else t)(jnp.asarray(a)))
    B, Hq, Hkv, Sq, Sk, D = 2, 32, 32, 1, 8192, 128
    return {
        "q": _w((lambda *s: _rng.normal(s) * 0.8)(B, Hq, Sq, D)),
        "k": _w((lambda *s: _rng.normal(s) * 0.8)(B, Hkv, Sk, D)),
        "v": _w((lambda *s: _rng.normal(s) * 0.05)(B, Hkv, Sk, D)),
    }

def reference(q, k, v):
    B, Hq, Sq, D = q.shape
    Hkv = k.shape[1]
    rep = Hq // Hkv
    k = jnp.repeat(k, rep, axis=1)
    v = jnp.repeat(v, rep, axis=1)
    scale = D ** -0.5
    scores = jnp.einsum("bhqd,bhkd->bhqk", q, k) * scale
    p = _softmax(scores, axis=-1)
    return jnp.einsum("bhqk,bhkd->bhqd", p, v)
```

```python
import math

import jax
import jax.experimental.pallas as pl
import jax.experimental.pallas.tpu as pltpu
import jax.numpy as jnp
import numpy as np
from jax import lax

_G = 8
_T = 256
_SUB = 16
_NBUF = 6

_NT = (((1,), (1,)), ((), ()))


def _pick_rows(parts):
    row = lax.broadcasted_iota(jnp.int32, parts[0].shape, 0)
    bit = 1
    while len(parts) > 1:
        odd = (row & bit) != 0
        parts = [jnp.where(odd, parts[i + 1], parts[i]) for i in range(0, len(parts), 2)]
        bit *= 2
    return parts[0]


@jax.jit
def pallas_standalone__gqa_softmax__decode_kernel(
    q: jax.Array,
    k: jax.Array,
    v: jax.Array,
):
    batch, heads, sq, d = q.shape
    seq = k.shape[2]
    assert sq == 1 and k.shape == v.shape == (batch, heads, seq, d)
    bh = batch * heads
    assert bh % _G == 0 and seq % _T == 0 and d == 128
    n_groups, n_chunks, n_pieces = bh // _G, seq // _T, _T // _SUB
    n_steps = n_groups * n_chunks
    scale_log2e = d**-0.5 * math.log2(math.e)
    lowest = float(np.finfo(np.float32).min)

    def kernel(q_hbm, k_hbm, v_hbm, o_hbm, kv_buf, kv_sem, q_buf, o_buf, q_sem, o_sem):
        def start_piece(step, slot, j):
            group, chunk = step // n_chunks, step % n_chunks
            key0 = pl.multiple_of(chunk * _T + j * _SUB, _SUB)
            for which, src in enumerate((k_hbm, v_hbm)):
                pltpu.make_async_copy(
                    src.at[pl.ds(group * _G, _G), pl.ds(key0, _SUB)],
                    kv_buf.at[slot, which, :, pl.ds(j * _SUB, _SUB)],
                    kv_sem.at[slot],
                ).start(priority=1 - which)

        q_copy = pltpu.make_async_copy(q_hbm, q_buf, q_sem)
        q_copy.start()

        def prologue(step, carry):
            for j in range(n_pieces):
                start_piece(step, step, j)
            return carry

        lax.fori_loop(0, _NBUF - 1, prologue, 0)
        q_copy.wait()

        def group_body(group, carry):
            rows = pl.ds(pl.multiple_of(group * _G, _G), _G)
            qg = q_buf[rows, :]

            def chunk_body(chunk, state):
                m, l, acc = state
                step = group * n_chunks + chunk
                slot = lax.rem(step, _NBUF)
                ahead = step + _NBUF - 1
                pltpu.make_async_copy(kv_buf.at[slot], kv_buf.at[slot], kv_sem.at[slot]).wait()

                def refill(tile):
                    for j in range(n_pieces):
                        if j * 2 * _G // n_pieces == tile:

                            @pl.when(ahead < n_steps)
                            def _():
                                start_piece(ahead, lax.rem(ahead, _NBUF), j)

                scores = []
                for h in range(_G):
                    refill(h)
                    scores.append(
                        lax.dot_general(qg, kv_buf[slot, 0, h], _NT, preferred_element_type=jnp.float32)
                    )
                s = _pick_rows(scores)
                m_new = jnp.maximum(m, jnp.max(s, axis=1, keepdims=True))
                alpha = jnp.exp2((m - m_new) * scale_log2e)
                p = jnp.exp2((s - m_new) * scale_log2e)
                l = alpha * l + sum(p[:, i : i + 128] for i in range(0, _T, 128))
                p = p.astype(v.dtype)
                outs = []
                for h in range(_G):
                    refill(_G + h)
                    outs.append(jnp.dot(p, kv_buf[slot, 1, h], preferred_element_type=jnp.float32))
                return m_new, l, alpha * acc + _pick_rows(outs)

            init = (
                jnp.full((_G, 1), lowest, jnp.float32),
                jnp.zeros((_G, 128), jnp.float32),
                jnp.zeros((_G, d), jnp.float32),
            )
            _, l, acc = lax.fori_loop(0, n_chunks, chunk_body, init)
            o_buf[rows, :] = (acc / jnp.sum(l, axis=1, keepdims=True)).astype(o_buf.dtype)
            return carry

        lax.fori_loop(0, n_groups, group_body, 0)
        o_copy = pltpu.make_async_copy(o_buf, o_hbm, o_sem)
        o_copy.start()
        o_copy.wait()

    out = pl.pallas_call(
        kernel,
        out_shape=jax.ShapeDtypeStruct((bh, d), q.dtype),
        in_specs=[pl.BlockSpec(memory_space=pl.ANY)] * 3,
        out_specs=pl.BlockSpec(memory_space=pl.ANY),
        scratch_shapes=[
            pltpu.VMEM((_NBUF, 2, _G, _T, d), k.dtype),
            pltpu.SemaphoreType.DMA((_NBUF,)),
            pltpu.VMEM((bh, d), q.dtype),
            pltpu.VMEM((bh, d), q.dtype),
            pltpu.SemaphoreType.DMA(()),
            pltpu.SemaphoreType.DMA(()),
        ],
        compiler_params=pltpu.CompilerParams(vmem_limit_bytes=32 * 1024 * 1024),
    )(q.reshape(bh, d), k.reshape(bh, seq, d), v.reshape(bh, seq, d))
    return out.reshape(q.shape)
```

```python
import math

import jax
import jax.experimental.pallas as pl
import jax.experimental.pallas.tpu as pltpu
import jax.numpy as jnp
import numpy as np
from jax import lax

_HEADS = 4
_ROWS = 2 * _HEADS
_T = 256
_SUB = 64
_NBUF = 4

_NT = (((1,), (1,)), ((), ()))


def _pick_rows(parts):
    row = lax.broadcasted_iota(jnp.int32, parts[0].shape, 0)
    bit = 1
    while len(parts) > 1:
        odd = (row & bit) != 0
        parts = [jnp.where(odd, parts[i + 1], parts[i]) for i in range(0, len(parts), 2)]
        bit *= 2
    return parts[0]


@jax.jit
def pallas_standalone__gqa_softmax__decode_kernel(
    q: jax.Array,
    k: jax.Array,
    v: jax.Array,
):
    batch, heads, sq, d = q.shape
    seq = k.shape[2]
    assert sq == 1 and k.shape == v.shape == (batch, heads, seq, d)
    bh, half = batch * heads, seq // 2
    assert bh % _ROWS == 0 and seq % (2 * _T) == 0 and d == 128
    n_groups, n_chunks = bh // _HEADS, half // _T
    n_steps = n_groups * n_chunks
    scale_log2e = d**-0.5 * math.log2(math.e)
    lowest = float(np.finfo(np.float32).min)
    pieces = [
        (h, f, key)
        for key in range(0, _T, _SUB)
        for h in range(0, _HEADS, 2)
        for f in range(2)
    ]

    def kernel(q_hbm, k_hbm, v_hbm, o_hbm, kv_buf, kv_sem, q_buf, o_buf, q_sem, o_sem):
        def start_piece(step, slot, piece):
            h, f, key = piece
            group, chunk = step // n_chunks, step % n_chunks
            key0 = pl.multiple_of(chunk * _T + key, _SUB)
            for which, src in enumerate((k_hbm, v_hbm)):
                pltpu.make_async_copy(
                    src.at[pl.ds(group * _HEADS + h, 2), f, pl.ds(key0, _SUB)],
                    kv_buf.at[slot, which, pl.ds(h, 2), f, pl.ds(key, _SUB)],
                    kv_sem.at[2 * slot + which],
                ).start(priority=which)

        def wait_slot(slot, which):
            buf = kv_buf.at[slot, which]
            pltpu.make_async_copy(buf, buf, kv_sem.at[2 * slot + which]).wait()

        def prologue(step, carry):
            for piece in pieces:
                start_piece(step, step, piece)
            return carry

        q_copy = pltpu.make_async_copy(q_hbm, q_buf, q_sem)
        q_copy.start()
        lax.fori_loop(0, _NBUF - 1, prologue, 0)
        q_copy.wait()
        row = lax.broadcasted_iota(jnp.int32, (_ROWS, d), 0)

        def group_body(group, o_prev):
            tile = pl.ds(pl.multiple_of((group // 2) * _ROWS, _ROWS), _ROWS)
            q8 = q_buf[tile, :].astype(jnp.float32)
            in_place = (row < _HEADS) == (group % 2 == 0)
            qg = jnp.where(in_place, q8, pltpu.roll(q8, _HEADS, 0)).astype(q.dtype)

            def chunk_body(chunk, state):
                m, l, acc = state
                step = group * n_chunks + chunk
                slot = lax.rem(step, _NBUF)
                ahead = step + _NBUF - 1

                def refill(i):
                    @pl.when(ahead < n_steps)
                    def _():
                        start_piece(ahead, lax.rem(ahead, _NBUF), pieces[i])

                per_tile = len(pieces) // (2 * _ROWS)
                wait_slot(slot, 0)
                scores = []
                for r in range(_ROWS):
                    for i in range(per_tile):
                        refill(r * per_tile + i)
                    kt = kv_buf[slot, 0, r % _HEADS, r // _HEADS]
                    scores.append(lax.dot_general(qg, kt, _NT, preferred_element_type=jnp.float32))
                s = _pick_rows(scores)
                m_new = jnp.maximum(m, jnp.max(s, axis=1, keepdims=True))
                alpha = jnp.exp2((m - m_new) * scale_log2e)
                p = jnp.exp2((s - m_new) * scale_log2e)
                l = alpha * l + sum(p[:, i : i + 128] for i in range(0, _T, 128))
                p = p.astype(v.dtype)
                wait_slot(slot, 1)
                outs = []
                for r in range(_ROWS):
                    for i in range(per_tile):
                        refill((_ROWS + r) * per_tile + i)
                    vt = kv_buf[slot, 1, r % _HEADS, r // _HEADS]
                    outs.append(jnp.dot(p, vt, preferred_element_type=jnp.float32))
                return m_new, l, alpha * acc + _pick_rows(outs)

            init = (
                jnp.full((_ROWS, 1), lowest, jnp.float32),
                jnp.zeros((_ROWS, 128), jnp.float32),
                jnp.zeros((_ROWS, d), jnp.float32),
            )
            m, l, acc = lax.fori_loop(0, n_chunks, chunk_body, init)
            m = jnp.broadcast_to(m, (_ROWS, d))
            w = jnp.exp2((m - jnp.maximum(m, pltpu.roll(m, _HEADS, 0))) * scale_log2e)
            lw = w * jnp.sum(l, axis=1, keepdims=True)
            aw = acc * (w / (lw + pltpu.roll(lw, _HEADS, 0)))
            o = aw + pltpu.roll(aw, _HEADS, 0)
            o_buf[tile, :] = jnp.where(row < _HEADS, o_prev, o).astype(o_buf.dtype)
            return o

        lax.fori_loop(0, n_groups, group_body, jnp.zeros((_ROWS, d), jnp.float32))
        o_copy = pltpu.make_async_copy(o_buf, o_hbm, o_sem)
        o_copy.start()
        o_copy.wait()

    out = pl.pallas_call(
        kernel,
        out_shape=jax.ShapeDtypeStruct((bh, d), q.dtype),
        in_specs=[pl.BlockSpec(memory_space=pl.ANY)] * 3,
        out_specs=pl.BlockSpec(memory_space=pl.ANY),
        scratch_shapes=[
            pltpu.VMEM((_NBUF, 2, _HEADS, 2, _T, d), k.dtype),
            pltpu.SemaphoreType.DMA((2 * _NBUF,)),
            pltpu.VMEM((bh, d), q.dtype),
            pltpu.VMEM((bh, d), q.dtype),
            pltpu.SemaphoreType.DMA(()),
            pltpu.SemaphoreType.DMA(()),
        ],
        compiler_params=pltpu.CompilerParams(
            vmem_limit_bytes=32 * 1024 * 1024,
            disable_bounds_checks=True,
            disable_semaphore_checks=True,
        ),
    )(q.reshape(bh, d), k.reshape(bh, 2, half, d), v.reshape(bh, 2, half, d))
    return out.reshape(q.shape)
```

```python
import math

import jax
import jax.experimental.pallas as pl
import jax.experimental.pallas.tpu as pltpu
import jax.numpy as jnp
import numpy as np
from jax import lax

_HEADS = 4
_ROWS = 2 * _HEADS
_KEYS = 256
_COPY_KEYS = 64
_SLOTS = 4
_LOW_FIRST = 14

_HEAD_PAIRS = [(h, 2, f, 1) for h in (0, 2) for f in (0, 1)]
_HALF_PAIRS = [(h, 1, 0, 2) for h in range(_HEADS)]
_COPIES = [(*p, k) for k in range(0, _KEYS, _COPY_KEYS) for p in _HEAD_PAIRS]
_WRAP_COPIES = [(*p, k) for k in range(0, _KEYS, _COPY_KEYS) for p in _HALF_PAIRS]
_TAIL_PARTS = [(0, 4, 0, 128), (0, 2, 128, 128), (2, 2, 128, 128)]
_TAIL_COPIES = [
    ((*p, k), part)
    for part, (h0, nh, k0, nk) in enumerate(_TAIL_PARTS)
    for k in range(k0, k0 + nk, _COPY_KEYS)
    for p in _HEAD_PAIRS
    if h0 <= p[0] < h0 + nh
]

_CONTRACT_LAST = (((1,), (1,)), ((), ()))
_K, _V = 0, 1


def _pick_rows(parts):
    row = lax.broadcasted_iota(jnp.int32, next(iter(parts.values())).shape, 0)
    bit = 1
    while len(parts) > 1:
        merged = {}
        for r in sorted(parts):
            key = r & ~bit
            if key in merged:
                merged[key] = jnp.where((row & bit) != 0, parts[r], merged[key])
            else:
                merged[key] = parts[r]
        parts, bit = merged, 2 * bit
    return next(iter(parts.values()))


@jax.jit
def pallas_standalone__gqa_softmax__decode_kernel(
    q: jax.Array,
    k: jax.Array,
    v: jax.Array,
):
    batch, heads, q_len, d = q.shape
    seq = k.shape[2]
    n_heads, half = batch * heads, seq // 2
    assert q_len == 1 and d == 128 and k.shape == v.shape == (batch, heads, seq, d)
    assert n_heads % _ROWS == 0 and n_heads > _ROWS
    assert seq % (2 * _KEYS) == 0 and half // _KEYS >= _SLOTS
    n_chunks = half // _KEYS
    last = (n_heads // _HEADS) * n_chunks - 1
    last_slot = last % _SLOTS
    scale_log2e = d**-0.5 * math.log2(math.e)
    lowest = float(np.finfo(np.float32).min)

    def kernel(
        q_hbm, k_hbm, v_hbm, o_hbm,
        kv_buf, q_buf, q_rot, o_rot, o_buf,
        kv_sem, tail_sem, io_sem,
    ):
        def start_copy(which, step, slot, copy, sem, priority):
            h, nh, f, nf, key = copy
            head = (step // n_chunks * _HEADS + h - 1) % n_heads
            src_key = step % n_chunks * _KEYS + key
            if not isinstance(src_key, int):
                src_key = pl.multiple_of(src_key, _COPY_KEYS)
            src = (k_hbm, v_hbm)[which]
            pltpu.make_async_copy(
                src.at[pl.ds(head, nh), pl.ds(f, nf), pl.ds(src_key, _COPY_KEYS)],
                kv_buf.at[slot, which, pl.ds(h, nh), pl.ds(f, nf), pl.ds(key, _COPY_KEYS)],
                sem,
            ).start(priority=priority)

        def start_kv(step, slot, copy, k_priority=0):
            start_copy(_K, step, slot, copy, kv_sem.at[2 * slot + _K], k_priority)
            start_copy(_V, step, slot, copy, kv_sem.at[2 * slot + _V], 1)

        def refill(step, lo, hi):
            slot = lax.rem(step, _SLOTS)

            @pl.when(step < n_chunks)
            def _():
                for copy in _WRAP_COPIES[lo:hi]:
                    start_kv(step, slot, copy)

            @pl.when((step >= n_chunks) & (step < last))
            def _():
                for copy in _COPIES[lo:hi]:
                    start_kv(step, slot, copy)

            @pl.when(step == last)
            def _():
                for k_copy, (v_copy, part) in zip(_COPIES[lo:hi], _TAIL_COPIES[lo:hi]):
                    start_copy(_K, last, last_slot, k_copy, kv_sem.at[2 * last_slot + _K], 0)
                    start_copy(_V, last, last_slot, v_copy, tail_sem.at[part], 1)

        def wait_filled(buf, sem):
            pltpu.make_async_copy(buf, buf, sem).wait()

        def wait_slot(slot, which):
            wait_filled(kv_buf.at[slot, which], kv_sem.at[2 * slot + which])

        def tile_of(group):
            start = group // 2 * _ROWS
            if not isinstance(start, int):
                start = pl.multiple_of(start, _ROWS)
            return pl.ds(start, _ROWS)

        def other_half(x):
            return pltpu.roll(x, _HEADS, 0)

        def scores(step, slot):
            group = step // n_chunks
            q8 = q_rot[tile_of(group), :]
            in_place = (row < _HEADS) == (group % 2 == 0)
            qg = jnp.where(in_place, q8, other_half(q8)).astype(q.dtype)
            return _pick_rows({
                r: lax.dot_general(
                    qg,
                    kv_buf[slot, _K, r % _HEADS, r // _HEADS],
                    _CONTRACT_LAST,
                    preferred_element_type=jnp.float32,
                )
                for r in range(_ROWS)
            })

        def softmax_step(s, m, l):
            m_new = jnp.maximum(m, jnp.max(s, axis=1, keepdims=True))
            alpha = jnp.exp2((m - m_new) * scale_log2e)
            p = jnp.exp2((s - m_new) * scale_log2e)
            l_new = alpha * l + sum(p[:, i : i + 128] for i in range(0, _KEYS, 128))
            return m_new, l_new, alpha, p.astype(v.dtype)

        def weighted_values(p, slot, rows=range(_ROWS), k0=0, nk=_KEYS):
            return _pick_rows({
                r: jnp.dot(
                    p[:, k0 : k0 + nk],
                    kv_buf[slot, _V, r % _HEADS, r // _HEADS, pl.ds(k0, nk)],
                    preferred_element_type=jnp.float32,
                )
                for r in range(_ROWS)
            })

        def merge_weights(m, l):
            m = jnp.broadcast_to(m, (_ROWS, d))
            w = jnp.exp2((m - jnp.maximum(m, other_half(m))) * scale_log2e)
            lw = w * jnp.sum(l, axis=1, keepdims=True)
            return w / (lw + other_half(lw))

        q_copy = pltpu.make_async_copy(q_hbm, q_buf, io_sem.at[0])
        q_copy.start()
        for i, copy in enumerate(_WRAP_COPIES):
            start_kv(0, 0, copy, k_priority=int(i < _LOW_FIRST))

        def prologue(step, carry):
            for copy in _WRAP_COPIES:
                start_kv(step, step, copy)
            return carry

        lax.fori_loop(1, _SLOTS - 1, prologue, 0)

        row = lax.broadcasted_iota(jnp.int32, (_ROWS, d), 0)
        o_rot[...] = jnp.zeros(o_rot.shape, o_rot.dtype)
        q_copy.wait()
        q_rot[...] = pltpu.roll(q_buf[...].astype(jnp.float32), 1, 0)
        wait_slot(0, _K)
        first = softmax_step(
            scores(0, 0),
            jnp.full((_ROWS, 1), lowest, jnp.float32),
            jnp.zeros((_ROWS, 128), jnp.float32),
        )

        def body(step, state):
            m, l, alpha, p, acc = state
            slot, next_slot = lax.rem(step, _SLOTS), lax.rem(step + 1, _SLOTS)
            ahead = step + _SLOTS - 1
            wait_slot(next_slot, _K)
            refill(ahead, 0, len(_COPIES) // 2)
            s = scores(step + 1, next_slot)
            wait_slot(slot, _V)
            group_ends = (step + 1) % n_chunks == 0
            following = softmax_step(
                s, jnp.where(group_ends, lowest, m), jnp.where(group_ends, 0.0, l)
            )
            refill(ahead, len(_COPIES) // 2, len(_COPIES))
            new = weighted_values(p, slot)
            acc = jnp.where(step % n_chunks == 0, new, alpha * acc + new)

            @pl.when(group_ends)
            def _():
                group = step // n_chunks
                part = acc * merge_weights(m, l)
                keep = (row < _HEADS) & (group % 2 == 1)
                o_rot[tile_of(group), :] = jnp.where(
                    keep, o_rot[tile_of(group), :], part + other_half(part)
                )

            return (*following, acc)

        m, l, alpha, p, acc = lax.fori_loop(
            0, last, body, (*first, jnp.zeros((_ROWS, d), jnp.float32))
        )

        early, late = pl.ds(0, n_heads - _ROWS), pl.ds(n_heads - _ROWS, _ROWS)
        early_copy = pltpu.make_async_copy(o_buf.at[early], o_hbm.at[early], io_sem.at[1])
        late_copy = pltpu.make_async_copy(o_buf.at[late], o_hbm.at[late], io_sem.at[2])
        acc = alpha * acc
        for part, (h0, nh, k0, nk) in enumerate(_TAIL_PARTS):
            wait_filled(
                kv_buf.at[last_slot, _V, pl.ds(h0, nh), :, pl.ds(k0, nk)], tail_sem.at[part]
            )
            if part == 0:
                done = pltpu.roll(o_rot[...], n_heads - 1, 0)
                o_buf[...] = done.astype(o_buf.dtype)
                early_copy.start()
                weights = merge_weights(m, l)
            rows = [r for r in range(_ROWS) if h0 <= r % _HEADS < h0 + nh]
            new = weighted_values(p, last_slot, rows, k0, nk)
            if nh < _HEADS:
                head = row & (_HEADS - 1)
                new = jnp.where((head >= h0) & (head < h0 + nh), new, 0.0)
            acc = acc + new
        part = acc * weights
        merged = pltpu.roll(part, _HEADS - 1, 0) + pltpu.roll(part, _ROWS - 1, 0)
        mine = (row >= _HEADS - 1) & (row < _ROWS - 1)
        o_buf[late, :] = jnp.where(mine, merged, done[n_heads - _ROWS :]).astype(o_buf.dtype)
        late_copy.start()
        early_copy.wait()
        late_copy.wait()

    out = pl.pallas_call(
        kernel,
        out_shape=jax.ShapeDtypeStruct((n_heads, d), q.dtype),
        in_specs=[pl.BlockSpec(memory_space=pl.ANY)] * 3,
        out_specs=pl.BlockSpec(memory_space=pl.ANY),
        scratch_shapes=[
            pltpu.VMEM((_SLOTS, 2, _HEADS, 2, _KEYS, d), k.dtype),
            pltpu.VMEM((n_heads, d), q.dtype),
            pltpu.VMEM((n_heads, d), jnp.float32),
            pltpu.VMEM((n_heads, d), jnp.float32),
            pltpu.VMEM((n_heads, d), q.dtype),
            pltpu.SemaphoreType.DMA((2 * _SLOTS,)),
            pltpu.SemaphoreType.DMA((len(_TAIL_PARTS),)),
            pltpu.SemaphoreType.DMA((3,)),
        ],
        compiler_params=pltpu.CompilerParams(disable_semaphore_checks=True),
    )(
        q.reshape(n_heads, d),
        k.reshape(n_heads, 2, half, d),
        v.reshape(n_heads, 2, half, d),
    )
    return out.reshape(q.shape)
```

```python
import math

import jax
import jax.experimental.pallas as pl
import jax.experimental.pallas.tpu as pltpu
import jax.numpy as jnp
import numpy as np
from jax import lax

_HEADS = 4
_ROWS = 2 * _HEADS
_KEYS = 256
_COPY_KEYS = 64
_SLOTS = 4
_LOW_FIRST = 14

_HEAD_PAIRS = [(h, 2, f, 1) for h in (0, 2) for f in (0, 1)]
_HALF_PAIRS = [(h, 1, 0, 2) for h in range(_HEADS)]
_COPIES = [(*p, k) for k in range(0, _KEYS, _COPY_KEYS) for p in _HEAD_PAIRS]
_WRAP_COPIES = [(*p, k) for k in range(0, _KEYS, _COPY_KEYS) for p in _HALF_PAIRS]
_TAIL_PARTS = [(0, 4, 0, 128), (0, 2, 128, 128), (2, 2, 128, 128)]
_TAIL_COPIES = [
    ((*p, k), part)
    for part, (h0, nh, k0, nk) in enumerate(_TAIL_PARTS)
    for k in range(k0, k0 + nk, _COPY_KEYS)
    for p in _HEAD_PAIRS
    if h0 <= p[0] < h0 + nh
]

_CONTRACT_LAST = (((1,), (1,)), ((), ()))
_K, _V = 0, 1


def _pick_rows(parts):
    row = lax.broadcasted_iota(jnp.int32, next(iter(parts.values())).shape, 0)
    bit = 1
    while len(parts) > 1:
        merged = {}
        for r in sorted(parts):
            key = r & ~bit
            if key in merged:
                merged[key] = jnp.where((row & bit) != 0, parts[r], merged[key])
            else:
                merged[key] = parts[r]
        parts, bit = merged, 2 * bit
    return next(iter(parts.values()))


@jax.jit
def pallas_standalone__gqa_softmax__decode_kernel(
    q: jax.Array,
    k: jax.Array,
    v: jax.Array,
):
    batch, heads, q_len, d = q.shape
    seq = k.shape[2]
    n_heads, half = batch * heads, seq // 2
    assert q_len == 1 and d == 128 and k.shape == v.shape == (batch, heads, seq, d)
    assert n_heads % _ROWS == 0 and n_heads > _ROWS
    assert seq % (2 * _KEYS) == 0 and half // _KEYS >= _SLOTS
    n_chunks = half // _KEYS
    last = (n_heads // _HEADS) * n_chunks - 1
    last_slot = last % _SLOTS
    scale_log2e = d**-0.5 * math.log2(math.e)
    lowest = float(np.finfo(np.float32).min)

    def kernel(
        q_hbm, k_hbm, v_hbm, o_hbm,
        kv_buf, q_buf, q_rot, o_rot, o_buf,
        kv_sem, tail_sem, io_sem,
    ):
        row = lax.broadcasted_iota(jnp.int32, (_ROWS, d), 0)

        def start_copy(which, step, slot, copy, sem, priority):
            h, nh, f, nf, key = copy
            head = (step // n_chunks * _HEADS + h - 1) % n_heads
            src_key = step % n_chunks * _KEYS + key
            if not isinstance(src_key, int):
                src_key = pl.multiple_of(src_key, _COPY_KEYS)
            src = (k_hbm, v_hbm)[which]
            pltpu.make_async_copy(
                src.at[pl.ds(head, nh), pl.ds(f, nf), pl.ds(src_key, _COPY_KEYS)],
                kv_buf.at[slot, which, pl.ds(h, nh), pl.ds(f, nf), pl.ds(key, _COPY_KEYS)],
                sem,
            ).start(priority=priority)

        def start_kv(step, slot, copy, k_priority=0):
            start_copy(_K, step, slot, copy, kv_sem.at[2 * slot + _K], k_priority)
            start_copy(_V, step, slot, copy, kv_sem.at[2 * slot + _V], 1)

        def refill(step, lo, hi):
            slot = lax.rem(step, _SLOTS)

            @pl.when(step < n_chunks)
            def _():
                for copy in _WRAP_COPIES[lo:hi]:
                    start_kv(step, slot, copy)

            @pl.when((step >= n_chunks) & (step < last))
            def _():
                for copy in _COPIES[lo:hi]:
                    start_kv(step, slot, copy)

            @pl.when(step == last)
            def _():
                for k_copy, (v_copy, part) in zip(_COPIES[lo:hi], _TAIL_COPIES[lo:hi]):
                    start_copy(_K, last, last_slot, k_copy, kv_sem.at[2 * last_slot + _K], 0)
                    start_copy(_V, last, last_slot, v_copy, tail_sem.at[part], 1)

        def wait_filled(buf, sem):
            pltpu.make_async_copy(buf, buf, sem).wait()

        def wait_slot(slot, which):
            wait_filled(kv_buf.at[slot, which], kv_sem.at[2 * slot + which])

        def tile_of(group):
            start = group // 2 * _ROWS
            if not isinstance(start, int):
                start = pl.multiple_of(start, _ROWS)
            return pl.ds(start, _ROWS)

        def other_half(x):
            return pltpu.roll(x, _HEADS, 0)

        def scores(step, slot):
            group = step // n_chunks
            q8 = q_rot[tile_of(group), :]
            in_place = (row < _HEADS) == (group % 2 == 0)
            qg = jnp.where(in_place, q8, other_half(q8)).astype(q.dtype)
            return _pick_rows({
                r: lax.dot_general(
                    qg,
                    kv_buf[slot, _K, r % _HEADS, r // _HEADS],
                    _CONTRACT_LAST,
                    preferred_element_type=jnp.float32,
                )
                for r in range(_ROWS)
            })

        def softmax_step(s, m, l):
            m_new = jnp.maximum(m, jnp.max(s, axis=1, keepdims=True))
            alpha = jnp.exp2((m - m_new) * scale_log2e)
            p = jnp.exp2((s - m_new) * scale_log2e)
            l_new = alpha * l + sum(p[:, i : i + 128] for i in range(0, _KEYS, 128))
            return m_new, l_new, alpha, p.astype(v.dtype)

        def weighted_values(p, slot, rows=range(_ROWS), k0=0, nk=_KEYS):
            return _pick_rows({
                r: jnp.dot(
                    p[:, k0 : k0 + nk],
                    kv_buf[slot, _V, r % _HEADS, r // _HEADS, pl.ds(k0, nk)],
                    preferred_element_type=jnp.float32,
                )
                for r in rows
            })

        def merge_weights(m, l):
            m = jnp.broadcast_to(m, (_ROWS, d))
            w = jnp.exp2((m - jnp.maximum(m, other_half(m))) * scale_log2e)
            lw = w * jnp.sum(l, axis=1, keepdims=True)
            return w / (lw + other_half(lw))

        q_copy = pltpu.make_async_copy(q_hbm, q_buf, io_sem.at[0])
        q_copy.start()
        for i, copy in enumerate(_WRAP_COPIES):
            start_kv(0, 0, copy, k_priority=int(i < _LOW_FIRST))

        def prologue(step, carry):
            for copy in _WRAP_COPIES:
                start_kv(step, step, copy)
            return carry

        lax.fori_loop(1, _SLOTS - 1, prologue, 0)

        o_rot[...] = jnp.zeros(o_rot.shape, o_rot.dtype)
        q_copy.wait()
        q_rot[...] = pltpu.roll(q_buf[...].astype(jnp.float32), 1, 0)
        wait_slot(0, _K)
        first = softmax_step(
            scores(0, 0),
            jnp.full((_ROWS, 1), lowest, jnp.float32),
            jnp.zeros((_ROWS, 128), jnp.float32),
        )

        def body(step, state):
            m, l, alpha, p, acc = state
            slot, next_slot = lax.rem(step, _SLOTS), lax.rem(step + 1, _SLOTS)
            ahead = step + _SLOTS - 1
            wait_slot(next_slot, _K)
            refill(ahead, 0, len(_COPIES) // 2)
            s = scores(step + 1, next_slot)
            wait_slot(slot, _V)
            group_ends = (step + 1) % n_chunks == 0
            following = softmax_step(
                s, jnp.where(group_ends, lowest, m), jnp.where(group_ends, 0.0, l)
            )
            refill(ahead, len(_COPIES) // 2, len(_COPIES))
            new = weighted_values(p, slot)
            acc = jnp.where(step % n_chunks == 0, new, alpha * acc + new)

            @pl.when(group_ends)
            def _():
                group = step // n_chunks
                share = acc * merge_weights(m, l)
                keep = (row < _HEADS) & (group % 2 == 1)
                o_rot[tile_of(group), :] = jnp.where(
                    keep, o_rot[tile_of(group), :], share + other_half(share)
                )

            return (*following, acc)

        m, l, alpha, p, acc = lax.fori_loop(
            0, last, body, (*first, jnp.zeros((_ROWS, d), jnp.float32))
        )

        early, late = pl.ds(0, n_heads - _ROWS), pl.ds(n_heads - _ROWS, _ROWS)
        early_copy = pltpu.make_async_copy(o_buf.at[early], o_hbm.at[early], io_sem.at[1])
        late_copy = pltpu.make_async_copy(o_buf.at[late], o_hbm.at[late], io_sem.at[2])
        acc = alpha * acc
        for part, (h0, nh, k0, nk) in enumerate(_TAIL_PARTS):
            wait_filled(
                kv_buf.at[last_slot, _V, pl.ds(h0, nh), :, pl.ds(k0, nk)], tail_sem.at[part]
            )
            if part == 0:
                done = pltpu.roll(o_rot[...], n_heads - 1, 0)
                o_buf[...] = done.astype(o_buf.dtype)
                early_copy.start()
                weights = merge_weights(m, l)
            rows = [r for r in range(_ROWS) if h0 <= r % _HEADS < h0 + nh]
            new = weighted_values(p, last_slot, rows, k0, nk)
            if nh < _HEADS:
                head = row & (_HEADS - 1)
                new = jnp.where((head >= h0) & (head < h0 + nh), new, 0.0)
            acc = acc + new
        share = acc * weights
        merged = pltpu.roll(share, _HEADS - 1, 0) + pltpu.roll(share, _ROWS - 1, 0)
        mine = (row >= _HEADS - 1) & (row < _ROWS - 1)
        o_buf[late, :] = jnp.where(mine, merged, done[n_heads - _ROWS :]).astype(o_buf.dtype)
        late_copy.start()
        early_copy.wait()
        late_copy.wait()

    out = pl.pallas_call(
        kernel,
        out_shape=jax.ShapeDtypeStruct((n_heads, d), q.dtype),
        in_specs=[pl.BlockSpec(memory_space=pl.ANY)] * 3,
        out_specs=pl.BlockSpec(memory_space=pl.ANY),
        scratch_shapes=[
            pltpu.VMEM((_SLOTS, 2, _HEADS, 2, _KEYS, d), k.dtype),
            pltpu.VMEM((n_heads, d), q.dtype),
            pltpu.VMEM((n_heads, d), jnp.float32),
            pltpu.VMEM((n_heads, d), jnp.float32),
            pltpu.VMEM((n_heads, d), q.dtype),
            pltpu.SemaphoreType.DMA((2 * _SLOTS,)),
            pltpu.SemaphoreType.DMA((len(_TAIL_PARTS),)),
            pltpu.SemaphoreType.DMA((3,)),
        ],
        compiler_params=pltpu.CompilerParams(disable_semaphore_checks=True),
    )(
        q.reshape(n_heads, d),
        k.reshape(n_heads, 2, half, d),
        v.reshape(n_heads, 2, half, d),
    )
    return out.reshape(q.shape)
```

```python
import math

import jax
import jax.experimental.pallas as pl
import jax.experimental.pallas.tpu as pltpu
import jax.numpy as jnp
import numpy as np
from jax import lax

_HEADS = 4
_ROWS = 2 * _HEADS
_KEYS = 256
_COPY_KEYS = 64
_SLOTS = 4
_LEAD = 11
_LOW_FIRST = 14

_PAIRS = [(h, 2, f) for h in (0, 2) for f in (0, 1)]
_COPIES = [(*p, k) for k in range(0, _KEYS, _COPY_KEYS) for p in _PAIRS]
_WRAP_COPIES = [[c] if c[0] else [(0, 1, *c[2:]), (1, 1, *c[2:])] for c in _COPIES]
_TAIL_PARTS = [(0, 4, 0, 128), (0, 2, 128, 128), (2, 2, 128, 128)]
_TAIL_COPIES = [
    ((*p, k), part)
    for part, (h0, nh, k0, nk) in enumerate(_TAIL_PARTS)
    for k in range(k0, k0 + nk, _COPY_KEYS)
    for p in _PAIRS
    if h0 <= p[0] < h0 + nh
]

_CONTRACT_LAST = (((1,), (1,)), ((), ()))
_K, _V = 0, 1


def _pick_rows(parts):
    row = lax.broadcasted_iota(jnp.int32, next(iter(parts.values())).shape, 0)
    bit = 1
    while len(parts) > 1:
        merged = {}
        for r in sorted(parts):
            key = r & ~bit
            if key in merged:
                merged[key] = jnp.where((row & bit) != 0, parts[r], merged[key])
            else:
                merged[key] = parts[r]
        parts, bit = merged, 2 * bit
    return next(iter(parts.values()))


@jax.jit
def pallas_standalone__gqa_softmax__decode_kernel(
    q: jax.Array,
    k: jax.Array,
    v: jax.Array,
):
    batch, heads, q_len, d = q.shape
    seq = k.shape[2]
    n_heads, half = batch * heads, seq // 2
    assert q_len == 1 and d == 128 and k.shape == v.shape == (batch, heads, seq, d)
    assert n_heads % _ROWS == 0 and n_heads > _ROWS
    assert seq % (2 * _KEYS) == 0 and half // _KEYS >= _SLOTS
    n_groups, n_chunks = n_heads // _HEADS, half // _KEYS
    lead = min(_LEAD, n_chunks - 2)
    last = n_groups * n_chunks - 1
    last_slot = last % _SLOTS
    scale_log2e = d**-0.5 * math.log2(math.e)
    lowest = float(np.finfo(np.float32).min)

    def kernel(
        q_hbm, k_hbm, v_hbm, o_hbm,
        kv_buf, q_buf, q_rot, o_rot, first_group, o_early, o_late,
        kv_sem, tail_sem, io_sem,
    ):
        row = lax.broadcasted_iota(jnp.int32, (_ROWS, d), 0)

        def leading(step):
            ahead = step % n_chunks < lead
            return int(ahead) if isinstance(ahead, bool) else ahead.astype(jnp.int32)

        def position(r, step):
            if r >= _HEADS:
                return r - _HEADS, 1
            return (r + _HEADS - leading(step)) % _HEADS, 0

        def start_copy(which, step, slot, copy, sem, priority):
            h, nh, f, key = copy
            head = step // n_chunks * _HEADS + h + n_heads - 1
            if f == 0:
                head = head + leading(step)
            src_key = step % n_chunks * _KEYS + key
            if not isinstance(src_key, int):
                src_key = pl.multiple_of(src_key, _COPY_KEYS)
            src = (k_hbm, v_hbm)[which]
            pltpu.make_async_copy(
                src.at[pl.ds(head % n_heads, nh), f, pl.ds(src_key, _COPY_KEYS)],
                kv_buf.at[slot, which, pl.ds(h, nh), f, pl.ds(key, _COPY_KEYS)],
                sem,
            ).start(priority=priority)

        def start_kv(step, slot, copy, k_priority=0):
            start_copy(_K, step, slot, copy, kv_sem.at[2 * slot + _K], k_priority)
            start_copy(_V, step, slot, copy, kv_sem.at[2 * slot + _V], 1)

        def refill(step, lo, hi):
            slot = lax.rem(step, _SLOTS)

            @pl.when(step < n_chunks)
            def _():
                for copies in _WRAP_COPIES[lo:hi]:
                    for copy in copies:
                        start_kv(step, slot, copy)

            @pl.when((step >= n_chunks) & (step < last))
            def _():
                for copy in _COPIES[lo:hi]:
                    start_kv(step, slot, copy)

            @pl.when(step == last)
            def _():
                for k_copy, (v_copy, part) in zip(_COPIES[lo:hi], _TAIL_COPIES[lo:hi]):
                    start_copy(_K, last, last_slot, k_copy, kv_sem.at[2 * last_slot + _K], 0)
                    start_copy(_V, last, last_slot, v_copy, tail_sem.at[part], 1)

        def wait_filled(buf, sem):
            pltpu.make_async_copy(buf, buf, sem).wait()

        def wait_slot(slot, which):
            wait_filled(kv_buf.at[slot, which], kv_sem.at[2 * slot + which])

        def tile_of(group):
            start = group // 2 * _ROWS
            if not isinstance(start, int):
                start = pl.multiple_of(start, _ROWS)
            return pl.ds(start, _ROWS)

        def other_half(x):
            return pltpu.roll(x, _HEADS, 0)

        def queries(group):
            q8 = q_rot[tile_of(group), :]
            return jnp.where((row < _HEADS) == (group % 2 == 0), q8, other_half(q8))

        def scores(step, slot):
            group = step // n_chunks
            row0 = queries((group + leading(step)) % n_groups)
            qg = jnp.where(row == 0, row0, queries(group)).astype(q.dtype)
            return _pick_rows({
                r: lax.dot_general(
                    qg,
                    kv_buf[(slot, _K, *position(r, step))],
                    _CONTRACT_LAST,
                    preferred_element_type=jnp.float32,
                )
                for r in range(_ROWS)
            })

        def decay(m_old, m_new):
            return jnp.exp2((m_old - m_new) * scale_log2e)

        def softmax_step(s, m, l):
            m_new = jnp.maximum(m, jnp.max(s, axis=1, keepdims=True))
            alpha = decay(m, m_new)
            p = [decay(s[:, i : i + d], m_new) for i in range(0, _KEYS, d)]
            return m_new, alpha * l + sum(p), alpha, jnp.concatenate(p, 1).astype(v.dtype)

        def weighted_values(p, step, slot, rows=range(_ROWS), k0=0, nk=_KEYS):
            return _pick_rows({
                r: jnp.dot(
                    p[:, k0 : k0 + nk],
                    kv_buf[(slot, _V, *position(r, step), pl.ds(k0, nk))],
                    preferred_element_type=jnp.float32,
                )
                for r in rows
            })

        def merge_weights(m, l):
            w = decay(m, jnp.maximum(m, other_half(m)))
            lw = w * jnp.sum(l, axis=1, keepdims=True)
            return w / (lw + other_half(lw))

        def write_group(group, m, l, acc, mine):
            share = acc * merge_weights(m, l)
            tile = tile_of(group)
            o_rot[tile, :] = jnp.where(mine, share + other_half(share), o_rot[tile, :])

        q_copy = pltpu.make_async_copy(q_hbm, q_buf, io_sem.at[0])
        q_copy.start()
        for i, copy in enumerate(c for copies in _WRAP_COPIES for c in copies):
            start_kv(0, 0, copy, k_priority=int(i < _LOW_FIRST))

        def prologue(step, carry):
            for copies in _WRAP_COPIES:
                for copy in copies:
                    start_kv(step, step, copy)
            return carry

        lax.fori_loop(1, _SLOTS - 1, prologue, 0)

        o_rot[...] = jnp.zeros(o_rot.shape, o_rot.dtype)
        zero = o_rot[tile_of(0), :]
        q_copy.wait()
        q_rot[...] = pltpu.roll(q_buf[...].astype(jnp.float32), 1, 0)
        wait_slot(0, _K)
        start = softmax_step(scores(0, 0), zero + lowest, zero)

        def body(step, state):
            m, l, alpha, p, acc, parked_m, parked_l, parked_acc = state
            slot, next_slot = lax.rem(step, _SLOTS), lax.rem(step + 1, _SLOTS)
            chunk, next_chunk = step % n_chunks, (step + 1) % n_chunks
            ahead = step + _SLOTS - 1

            wait_slot(next_slot, _K)
            refill(ahead, 0, len(_COPIES) // 2)
            s = scores(step + 1, next_slot)
            wait_slot(slot, _V)
            swap = next_chunk == lead
            m_in = jnp.where(swap & (row == 0), parked_m, m)
            l_in = jnp.where(swap & (row == 0), parked_l, l)
            parked_m, parked_l = jnp.where(swap, m, parked_m), jnp.where(swap, l, parked_l)
            following = softmax_step(
                s,
                jnp.where(next_chunk == 0, lowest, m_in),
                jnp.where(next_chunk == 0, 0.0, l_in),
            )
            refill(ahead, len(_COPIES) // 2, len(_COPIES))
            new = weighted_values(p, step, slot)
            swap = chunk == lead
            acc_in = jnp.where(swap & (row == 0), parked_acc, acc)
            parked_acc = jnp.where(swap, acc, parked_acc)
            acc = jnp.where(chunk == 0, new, alpha * acc_in + new)

            @pl.when(next_chunk == 0)
            def _():
                group = step // n_chunks
                write_group(group, m, l, acc, (row < _HEADS) == (group % 2 == 0))

            @pl.when(step == n_chunks - 1)
            def _():
                first_group[0], first_group[1], first_group[2] = m, l, acc

            return (*following, acc, parked_m, parked_l, parked_acc)

        m, l, alpha, p, acc, parked_m, parked_l, parked_acc = lax.fori_loop(
            0, last, body, (*start, zero, zero + lowest, zero, zero)
        )

        split = n_heads - _ROWS
        early_copy = pltpu.make_async_copy(o_early, o_hbm.at[pl.ds(0, split)], io_sem.at[1])
        late_copy = pltpu.make_async_copy(o_late, o_hbm.at[pl.ds(split, _ROWS)], io_sem.at[2])
        acc = alpha * acc
        for part, (h0, nh, k0, nk) in enumerate(_TAIL_PARTS):
            wait_filled(
                kv_buf.at[last_slot, _V, pl.ds(h0, nh), :, pl.ds(k0, nk)], tail_sem.at[part]
            )
            if part == 0:
                m0, l0, acc0 = first_group[0], first_group[1], first_group[2]
                top = jnp.maximum(m0, parked_m)
                a, b = decay(m0, top), decay(parked_m, top)
                write_group(
                    0,
                    jnp.where(row == 0, top, m0),
                    jnp.where(row == 0, a * l0 + b * parked_l, l0),
                    jnp.where(row == 0, a * acc0 + b * parked_acc, acc0),
                    row < _HEADS,
                )
                done = pltpu.roll(o_rot[...], n_heads - 1, 0)
                o_early[...] = done[:split].astype(o_early.dtype)
                early_copy.start()
                weights = merge_weights(m, l)
            rows = [r for r in range(_ROWS) if h0 <= r % _HEADS < h0 + nh]
            new = weighted_values(p, last, last_slot, rows, k0, nk)
            if nh < _HEADS:
                head = row & (_HEADS - 1)
                new = jnp.where((head >= h0) & (head < h0 + nh), new, 0.0)
            acc = acc + new
        share = acc * weights
        merged = pltpu.roll(share, _HEADS - 1, 0) + pltpu.roll(share, _ROWS - 1, 0)
        mine = (row >= _HEADS - 1) & (row < _ROWS - 1)
        o_late[...] = jnp.where(mine, merged, done[split:]).astype(o_late.dtype)
        late_copy.start()
        early_copy.wait()
        late_copy.wait()

    out = pl.pallas_call(
        kernel,
        out_shape=jax.ShapeDtypeStruct((n_heads, d), q.dtype),
        in_specs=[pl.BlockSpec(memory_space=pl.ANY)] * 3,
        out_specs=pl.BlockSpec(memory_space=pl.ANY),
        scratch_shapes=[
            pltpu.VMEM((_SLOTS, 2, _HEADS, 2, _KEYS, d), k.dtype),
            pltpu.VMEM((n_heads, d), q.dtype),
            pltpu.VMEM((n_heads, d), jnp.float32),
            pltpu.VMEM((n_heads, d), jnp.float32),
            pltpu.VMEM((3, _ROWS, d), jnp.float32),
            pltpu.VMEM((n_heads - _ROWS, d), q.dtype),
            pltpu.VMEM((_ROWS, d), q.dtype),
            pltpu.SemaphoreType.DMA((2 * _SLOTS,)),
            pltpu.SemaphoreType.DMA((len(_TAIL_PARTS),)),
            pltpu.SemaphoreType.DMA((3,)),
        ],
        compiler_params=pltpu.CompilerParams(disable_semaphore_checks=True),
    )(
        q.reshape(n_heads, d),
        k.reshape(n_heads, 2, half, d),
        v.reshape(n_heads, 2, half, d),
    )
    return out.reshape(q.shape)
```
